```python
import jax
import jax.numpy as jnp

def _softmax(x, axis=-1):
    return jax.nn.softmax(x, axis=axis)
def _gelu(x):
    return jax.nn.gelu(x, approximate=True)
def _silu(x):
    return jax.nn.silu(x)
def _sigmoid(x):
    return jax.nn.sigmoid(x)
def _layernorm(x, axis=-1, eps=1e-5):
    m = jnp.mean(x, axis=axis, keepdims=True)
    v = jnp.var(x, axis=axis, keepdims=True)
    return (x - m) / jnp.sqrt(v + eps)
def _scatter_add(tgt, idx, src, axis=0):
    return tgt.at[idx].add(src)
def _segment_sum(src, seg, n):
    return jax.ops.segment_sum(src, seg, n)
class _Rng:
    def __init__(self, key):
        self._k = key
    def _next(self):
        self._k, sub = jax.random.split(self._k)
        return sub
    def normal(self, shape):
        return jax.random.normal(self._next(), shape, dtype=jnp.bfloat16)
    def randint(self, lo, hi, shape):
        return jax.random.randint(self._next(), shape, lo, hi, dtype=jnp.int32)
    def uniform(self, shape, lo=0.0, hi=1.0):
        return jax.random.uniform(self._next(), shape, jnp.bfloat16, lo, hi)
    def permutation(self, n):
        return jax.random.permutation(self._next(), n)


kernel_name = 'standalone__qk_norm__prompt'

def setup_inputs():
    _rng = _Rng(jax.random.key(int.from_bytes(__import__("os").urandom(4), "little")))
    _w = (lambda a: (lambda t: t.astype(jnp.bfloat16) if jnp.issubdtype(t.dtype, jnp.floating) else t)(jnp.asarray(a)))
    B, H, S, D = 2, 32, 2048, 1024
    Dh = D // H
    return {
        "q": _w((lambda *s: _rng.normal(s) * 0.05)(B, H, S, Dh)),
        "k": _w((lambda *s: _rng.normal(s) * 0.05)(B, H, S, Dh)),
        "v": _w((lambda *s: _rng.normal(s) * 0.05)(B, H, S, Dh)),
        "t": _w(jnp.abs((lambda *s: _rng.normal(s) * 0.05)(H)) + 1.0),
    }

def reference(q, k, v, t):
    eps = 1e-6
    qn = q / (jnp.sqrt((q * q).sum(axis=-1, keepdims=True)) + eps)
    kn = k / (jnp.sqrt((k * k).sum(axis=-1, keepdims=True)) + eps)
    logits = jnp.einsum('bhqd,bhkd->bhqk', qn, kn) * t[None, :, None, None]
    attn = _softmax(logits, axis=-1)
    return jnp.einsum('bhqk,bhkd->bhqd', attn, v)
```

```python
import functools

import jax
import jax.numpy as jnp
from jax import lax
import jax.experimental.pallas as pl
import jax.experimental.pallas.tpu as pltpu

_LOG2E = 1.4426950408889634
_EPS = 1e-6
_T_SAFE = 8.0
_G = 2
_BQ = 2048
_BK = 128
_NPIECE = 4

f32, bf16 = jnp.float32, jnp.bfloat16


def _unit_columns(x):
    return 1.0 / (jnp.sqrt(jnp.sum(x * x, axis=0, keepdims=True)) + _EPS)


def _q_piece(src, scale, dst, lo, hi):
    x = src[:, lo:hi].astype(f32)
    dst[:, lo:hi] = (x * (scale * _unit_columns(x))).astype(bf16)


def _k_piece(src, dst, r0, r1, *, n_chunks, chunk):
    parts = []
    for c in range(n_chunks):
        x = src[:, c * chunk + r0: c * chunk + r1].astype(f32)
        parts.append(x * _unit_columns(x))
    dst[r0:r1, :] = jnp.concatenate(parts, axis=0).T.astype(bf16)


def _prologue_pieces(q_src, k_src, scale, q_dst, k_dst, *, seq, n_chunks):
    chunk = seq // n_chunks
    qs = seq // _NPIECE
    kr = max(chunk // _NPIECE, 128)
    pieces = [functools.partial(_q_piece, q_src, scale, q_dst, i * qs, (i + 1) * qs)
              for i in range(_NPIECE)]
    pieces += [functools.partial(_k_piece, k_src, k_dst, r, r + kr,
                                 n_chunks=n_chunks, chunk=chunk)
               for r in range(0, chunk, kr)]
    return pieces


def _padded_q(qw, c, n_chunks):
    d, n = qw.shape
    parts = []
    if c > 0:
        parts.append(jnp.zeros((d * c, n), bf16))
    parts.append(qw)
    if c < n_chunks - 1:
        parts.append(jnp.zeros((d * (n_chunks - 1 - c), n), bf16))
    return jnp.concatenate(parts, axis=0) if len(parts) > 1 else qw


def _kernel(t_ref, q_cur, k_cur, q_nxt, k_nxt, v_cur, o_ref,
            q_a, k_a, q_b, k_b, safe_ref, *, seq, n_heads, n_chunks):
    step = pl.program_id(0)
    chunk = seq // n_chunks
    slots = [(q_a, k_a), (q_b, k_b)]
    nq, nk = seq // _BQ, seq // _BK

    def scale_of(head):
        return t_ref[head % n_heads] * _LOG2E

    def pieces_for(g):
        q_dst, k_dst = slots[(g + 1) % 2]
        q_src, k_src = ((q_cur.at[g + 1], k_cur.at[g + 1]) if g + 1 < _G
                        else (q_nxt.at[0], k_nxt.at[0]))
        return _prologue_pieces(q_src, k_src, scale_of(step * _G + g + 1), q_dst, k_dst,
                                seq=seq, n_chunks=n_chunks)

    @pl.when(step == 0)
    def _():
        t_max = lax.fori_loop(
            0, n_heads, lambda h, m: jnp.maximum(m, jnp.abs(t_ref[h])), jnp.float32(0.0))
        safe_ref[0] = (t_max <= _T_SAFE).astype(jnp.int32)
        for piece in _prologue_pieces(q_cur.at[0], k_cur.at[0], scale_of(0), q_a, k_a,
                                      seq=seq, n_chunks=n_chunks):
            piece()

    safe = safe_ref[0]

    @pl.when(safe == 1)
    def _():
        steps = [(g, j, kb) for g in range(_G) for j in range(nq) for kb in range(nk)]
        todo = {}
        for g in range(_G):
            for n, piece in enumerate(pieces_for(g)):
                todo.setdefault(g * nq * nk + 2 + n, []).append(piece)

        def qk(g, j, kb):
            q_s, k_s = slots[g % 2]
            c, off = divmod(kb * _BK, chunk)
            w = _padded_q(q_s[:, j * _BQ:(j + 1) * _BQ], c, n_chunks)
            return jnp.dot(k_s[off:off + _BK, :], w, preferred_element_type=f32)

        s_next = qk(*steps[0])
        acc = l_acc = None
        for n, (g, j, kb) in enumerate(steps):
            s = s_next
            if n + 1 < len(steps):
                s_next = qk(*steps[n + 1])
            p = jnp.exp2(s)
            l_part = jnp.sum(p.reshape(_BK // 8, 8, _BQ), axis=0)
            pv = jnp.dot(v_cur[g, :, kb * _BK:(kb + 1) * _BK], p.astype(bf16),
                         preferred_element_type=f32)
            l_acc = l_part if kb == 0 else l_acc + l_part
            acc = pv if kb == 0 else acc + pv
            if kb == nk - 1:
                l_sum = jnp.sum(l_acc, axis=0, keepdims=True)
                o_ref[g, :, j * _BQ:(j + 1) * _BQ] = (acc * (1.0 / l_sum)).astype(o_ref.dtype)
            for piece in todo.get(n, []):
                piece()

    @pl.when(safe != 1)
    def _():
        bq, bk = 256, chunk
        for g in range(_G):
            q_s, k_s = slots[g % 2]

            def q_block(j, carry, g=g, q_s=q_s, k_s=k_s):
                q0 = pl.multiple_of(j * bq, bq)
                qw = q_s[:, pl.ds(q0, bq)]

                def logits(c):
                    return jnp.dot(k_s[...], _padded_q(qw, c, n_chunks),
                                   preferred_element_type=f32)

                m = None
                for c in range(n_chunks):
                    m_c = jnp.max(logits(c), axis=0, keepdims=True)
                    m = m_c if m is None else jnp.maximum(m, m_c)
                acc = l_sum = None
                for c in range(n_chunks):
                    p = jnp.exp2(logits(c) - m)
                    l_c = jnp.sum(p, axis=0, keepdims=True)
                    pv = jnp.dot(v_cur[g, :, c * bk:(c + 1) * bk], p.astype(bf16),
                                 preferred_element_type=f32)
                    l_sum = l_c if l_sum is None else l_sum + l_c
                    acc = pv if acc is None else acc + pv
                o_ref[g, :, pl.ds(q0, bq)] = (acc * (1.0 / l_sum)).astype(o_ref.dtype)
                return carry

            lax.fori_loop(0, seq // bq, q_block, 0)
            for piece in pieces_for(g):
                piece()


@jax.jit
def pallas_standalone__qk_norm__prompt_kernel(
    q: jax.Array,
    k: jax.Array,
    v: jax.Array,
    t: jax.Array,
):
    b, h, s, d = q.shape
    n = b * h
    n_chunks = 128 // d
    assert n % _G == 0 and s % _BQ == 0 and (s // n_chunks) % 128 == 0

    def transposed(x):
        return jnp.transpose(x, (0, 1, 3, 2)).reshape(n, d, s)

    cur = pl.BlockSpec((_G, d, s), lambda i: (i, 0, 0))
    nxt = pl.BlockSpec((1, d, s), lambda i: (jnp.minimum((i + 1) * _G, n - 1), 0, 0))
    q_t, k_t, v_t = transposed(q), transposed(k), transposed(v)
    out = pl.pallas_call(
        functools.partial(_kernel, seq=s, n_heads=h, n_chunks=n_chunks),
        grid=(n // _G,),
        in_specs=[pl.BlockSpec(memory_space=pltpu.SMEM), cur, cur, nxt, nxt, cur],
        out_specs=cur,
        out_shape=jax.ShapeDtypeStruct((n, d, s), q.dtype),
        scratch_shapes=[
            pltpu.VMEM((d, s), bf16), pltpu.VMEM((s // n_chunks, 128), bf16),
            pltpu.VMEM((d, s), bf16), pltpu.VMEM((s // n_chunks, 128), bf16),
            pltpu.SMEM((1,), jnp.int32),
        ],
        compiler_params=pltpu.CompilerParams(
            dimension_semantics=("arbitrary",),
            vmem_limit_bytes=100 << 20,
            flags={"XLA_TPU_EVENLY_DISTRIBUTE_CRITICAL_NODES": True},
        ),
    )(t.astype(f32), q_t, k_t, q_t, k_t, v_t)
    return jnp.transpose(out.reshape(b, h, d, s), (0, 1, 3, 2))
```

```python
import functools

import jax
import jax.numpy as jnp
from jax import lax
import jax.experimental.pallas as pl
import jax.experimental.pallas.tpu as pltpu

_LOG2E = 1.4426950408889634
_EPS = 1e-6
_T_SAFE = 8.0
_G = 2
_BQ = 512
_BK = 128
_LOOK = 2
_VR = 16
_VSTEPS = (5, 10, 15)
_KB_PARTS = 2
_DMA_STEP = 8
_AHEAD = 3
_LANES = 128

f32, bf16, i32 = jnp.float32, jnp.bfloat16, jnp.int32


def _inv_norm(x):
    return 1.0 / (jnp.sqrt(jnp.sum(x * x, axis=0, keepdims=True)) + _EPS)


def _tie(never, token, operand):
    bits = jnp.where(never, pltpu.bitcast(token, i32), pltpu.bitcast(operand, i32))
    return pltpu.bitcast(bits, bf16)


def _prologue_parts(q_src, k_src, scale, slot, *, seq, dim, with_vpu=True):
    q_s, k_s, qf_s, kb_s = slot
    n_chunks = _LANES // dim
    chunk = seq // n_chunks

    def q_part(lo):
        x = q_src[:, lo:lo + _LANES].astype(f32)
        y = x * (scale() * _inv_norm(x))
        q_s[lo // _LANES] = y.astype(bf16)
        if with_vpu:
            qf_s[:, lo:lo + _LANES] = y
        return y[dim - 8:, :]

    def k_norm(state, r0, c):
        x = k_src[:, c * chunk + r0: c * chunk + r0 + _LANES].astype(f32)
        state[c] = x * _inv_norm(x)
        return state[c][dim - 8:, :]

    def k_transpose(state, r0):
        kt = jnp.concatenate([state.pop(c) for c in range(n_chunks)], axis=0).T
        state["kt"] = kt
        k_s[r0:r0 + _LANES, :] = kt.astype(bf16)
        return kt[_LANES - 8:, :]

    def k_broadcast(state, c, m, d0, d1):
        for d in range(d0, d1):
            col = c * dim + d
            val = jnp.broadcast_to(state["kt"][_BK - _VR:_BK, col:col + 1], (_VR, _LANES))
            kb_s[d, m * _VR:(m + 1) * _VR, :] = val
        return val[_VR - 8:, :]

    parts = [functools.partial(q_part, lo) for lo in range(0, seq, _LANES)]
    for r0 in range(0, chunk, _LANES):
        state = {}
        parts += [functools.partial(k_norm, state, r0, c) for c in range(n_chunks)]
        parts.append(functools.partial(k_transpose, state, r0))
        for c in range(n_chunks):
            step = (c * chunk + r0) // _BK
            if with_vpu and step in _VSTEPS:
                n = dim // _KB_PARTS
                parts += [functools.partial(k_broadcast, state, c, _VSTEPS.index(step),
                                            a * n, (a + 1) * n) for a in range(_KB_PARTS)]
    return parts


def _chunk_weights(qw, c, n_chunks):
    d, n = qw.shape
    parts = []
    if c > 0:
        parts.append(jnp.zeros((d * c, n), bf16))
    parts.append(qw)
    if c < n_chunks - 1:
        parts.append(jnp.zeros((d * (n_chunks - 1 - c), n), bf16))
    return jnp.concatenate(parts, axis=0) if len(parts) > 1 else qw


class _VpuLogits:
    def __init__(self, slot, q0, m, dim):
        self.qf_s, self.kb_s = slot[2], slot[3]
        self.q0, self.m = q0, m
        self.tiles = _BQ // _LANES
        self.todo = [(d, j) for d in range(dim) for j in range(self.tiles)]
        self.acc = [None] * self.tiles
        self.n_tokens = 0

    def advance(self, count):
        for d, j in self.todo[:count]:
            c0 = self.q0 + j * _LANES
            prod = self.kb_s[d, self.m * _VR:(self.m + 1) * _VR, :] * jnp.broadcast_to(
                self.qf_s[d:d + 1, c0:c0 + _LANES], (_VR, _LANES))
            self.acc[j] = prod if self.acc[j] is None else self.acc[j] + prod
        del self.todo[:count]

    def token(self):
        self.n_tokens += 1
        live = [a for a in self.acc if a is not None]
        half = self.n_tokens % 2
        return live[(self.n_tokens // 2) % len(live)][half * 8:(half + 1) * 8, :]

    def result(self):
        self.advance(len(self.todo))
        return jnp.concatenate(self.acc, axis=1)


class _Pacer:
    def __init__(self, jobs, n_slots):
        self.jobs = list(jobs)
        self.slots = n_slots
        self.rest = sum(len(job.todo) for job in self.jobs)

    def tie(self, never, operand):
        if self.rest <= 0 or self.slots <= 0:
            return operand
        count = -(-self.rest // self.slots)
        self.slots -= 1
        while count > 0 and self.jobs:
            job = self.jobs[0]
            n = min(count, len(job.todo))
            job.advance(n)
            count -= n
            self.rest -= n
            token = job.token() if (count == 0 or not job.todo) else None
            if not job.todo:
                self.jobs.pop(0)
            if count == 0:
                operand = _tie(never, token, operand)
        return operand


def _kernel(t_ref, q_hbm, k_hbm, v_hbm, o_hbm,
            q_a, k_a, qf_a, kb_a, q_b, k_b, qf_b, kb_b, zero_s, scale_s,
            q_v, k_v, v_v, o_v, sem_q, sem_k, sem_v, sem_o, *, n_heads):
    n, dim, seq = o_v.shape
    n_groups = n // _G
    n_chunks = _LANES // dim
    chunk = seq // n_chunks
    nq, nk = seq // _BQ, seq // _BK
    slots = [(q_a, k_a, qf_a, kb_a), (q_b, k_b, qf_b, kb_b)]

    def in_copies(c):
        src, dst, sem = jnp.minimum(c, n_groups - 1) * _G, c * _G, c % (_AHEAD + 1)
        return [pltpu.make_async_copy(hbm.at[pl.ds(src, _G)], vmem.at[pl.ds(dst, _G)],
                                      sems.at[sem])
                for hbm, vmem, sems in ((q_hbm, q_v, sem_q), (k_hbm, k_v, sem_k),
                                        (v_hbm, v_v, sem_v))]

    def out_copy(h):
        return pltpu.make_async_copy(o_v.at[pl.ds(h, 1)], o_hbm.at[pl.ds(h, 1)], sem_o.at[0])

    def start(copies):
        for cp in copies:
            cp.start()

    def wait(copies):
        for cp in copies:
            cp.wait()

    first = in_copies(0)
    start(first)
    for c in range(1, _AHEAD):
        start(in_copies(c))

    t_row = t_ref[...].astype(f32)
    safe = jnp.max(jnp.abs(t_row)) <= _T_SAFE
    t_pad = jnp.concatenate([t_row, jnp.zeros((1, _LANES - n_heads), f32)], axis=1)
    scale_s[...] = jnp.broadcast_to(t_pad * _LOG2E, (_LANES, _LANES)).T[:n_heads, :]
    zero_s[...] = jnp.zeros(zero_s.shape, i32)

    def scale_of(head):
        return lambda: scale_s[pl.ds(head % n_heads, 1), :]

    wait(first)

    def fast_group(i, carry):
        wait(in_copies(i + 1))
        never = zero_s[...] != 0
        steps = [(g, j, kb) for g in range(_G) for j in range(nq) for kb in range(nk)]

        tied = {}
        for g in range(_G):
            head = i * _G + g + 1
            src = head if g + 1 < _G else jnp.minimum(head, n - 1)
            parts = _prologue_parts(q_v.at[src], k_v.at[src], scale_of(head),
                                    slots[(g + 1) % 2], seq=seq, dim=dim)
            lo, hi = 1, nq * nk - _LOOK - 2
            for m, part in enumerate(parts):
                tied.setdefault(g * nq * nk + lo + (m * (hi - lo)) // len(parts),
                                []).append(part)

        jobs, pacers = {}, {}
        n_regs = sum((_BK - (_VR if kb in _VSTEPS else 0)) // 16 for kb in range(nk))
        for g in range(_G):
            for j in range(nq):
                for m, kb in enumerate(_VSTEPS):
                    jobs[g, j, kb] = _VpuLogits(slots[g % 2], j * _BQ, m, dim)
                pacers[g, j] = _Pacer([jobs[g, j, kb] for kb in _VSTEPS], n_regs)

        def qk(n_step):
            g, j, kb = steps[n_step]
            q_s, k_s = slots[g % 2][:2]
            c, off = divmod(kb * _BK, chunk)
            tiles = _BQ // _LANES
            qw = jnp.concatenate([q_s[j * tiles + a] for a in range(tiles)], axis=1)
            w = _chunk_weights(qw, c, n_chunks)
            tokens = [part() for part in tied.get(n_step, [])]
            regs = []
            for r in range((_BK - (_VR if kb in _VSTEPS else 0)) // 16):
                reg = pacers[g, j].tie(never, k_s[off + r * 16: off + (r + 1) * 16, :])
                if r < len(tokens):
                    reg = _tie(never, tokens[r], reg)
                regs.append(reg)
            return jnp.dot(jnp.concatenate(regs, axis=0), w, preferred_element_type=f32)

        pending = [qk(m) for m in range(_LOOK)]
        acc = l_acc = None
        for n_step, (g, j, kb) in enumerate(steps):
            if n_step + _LOOK < len(steps):
                pending.append(qk(n_step + _LOOK))
            s = pending.pop(0)
            if (g, j, kb) in jobs:
                s = jnp.concatenate([s, jobs[g, j, kb].result()], axis=0)
            p = jnp.exp2(s)
            l_part = jnp.sum(p.reshape(_BK // 8, 8, _BQ), axis=0)
            l_acc = l_part if kb == 0 else l_acc + l_part
            head = i * _G + g
            pv = jnp.dot(v_v[head, :, kb * _BK:(kb + 1) * _BK], p.astype(bf16),
                         preferred_element_type=f32)
            acc = pv if kb == 0 else acc + pv
            if kb == nk - 1:
                l_sum = jnp.sum(l_acc, axis=0, keepdims=True)
                o_v[head, :, j * _BQ:(j + 1) * _BQ] = (acc * (1.0 / l_sum)).astype(o_v.dtype)
                if j == nq - 1:
                    out_copy(head).start()
            if n_step == _DMA_STEP:
                start(in_copies(i + _AHEAD))
        return carry

    @pl.when(safe)
    def _():
        for part in _prologue_parts(q_v.at[0], k_v.at[0], scale_of(0), slots[0],
                                    seq=seq, dim=dim):
            part()
        lax.fori_loop(0, n_groups, fast_group, 0)

    def safe_group(i, carry):
        wait(in_copies(i + 1))
        start(in_copies(i + _AHEAD))
        q_s, k_s = slots[0][:2]

        def one_head(head, carry):
            for part in _prologue_parts(q_v.at[head], k_v.at[head], scale_of(head),
                                        slots[0], seq=seq, dim=dim, with_vpu=False):
                part()

            def q_tile(j, carry):
                qw = q_s[j]

                def logits(c):
                    return jnp.dot(k_s[...], _chunk_weights(qw, c, n_chunks),
                                   preferred_element_type=f32)

                m = None
                for c in range(n_chunks):
                    m_c = jnp.max(logits(c), axis=0, keepdims=True)
                    m = m_c if m is None else jnp.maximum(m, m_c)
                acc = l_sum = None
                for c in range(n_chunks):
                    p = jnp.exp2(logits(c) - m)
                    l_c = jnp.sum(p, axis=0, keepdims=True)
                    pv = jnp.dot(v_v[head, :, c * chunk:(c + 1) * chunk], p.astype(bf16),
                                 preferred_element_type=f32)
                    l_sum = l_c if l_sum is None else l_sum + l_c
                    acc = pv if acc is None else acc + pv
                q0 = pl.multiple_of(j * _LANES, _LANES)
                o_v[head, :, pl.ds(q0, _LANES)] = (acc * (1.0 / l_sum)).astype(o_v.dtype)
                return carry

            lax.fori_loop(0, seq // _LANES, q_tile, 0)
            out_copy(head).start()
            return carry

        return lax.fori_loop(i * _G, (i + 1) * _G, one_head, carry)

    @pl.when(jnp.logical_not(safe))
    def _():
        lax.fori_loop(0, n_groups, safe_group, 0)

    for c in range(n_groups + 1, n_groups + _AHEAD):
        wait(in_copies(c))
    pltpu.make_async_copy(o_v, o_hbm, sem_o.at[0]).wait()


@jax.jit
def pallas_standalone__qk_norm__prompt_kernel(
    q: jax.Array,
    k: jax.Array,
    v: jax.Array,
    t: jax.Array,
):
    b, h, s, d = q.shape
    n = b * h
    assert n % _G == 0 and s % _BQ == 0 and (s * d // _LANES) % _LANES == 0 and h <= _LANES

    def transposed(x):
        return jnp.transpose(x, (0, 1, 3, 2)).reshape(n, d, s)

    slot = [
        pltpu.VMEM((s // _LANES, d, _LANES), bf16),
        pltpu.VMEM((s * d // _LANES, _LANES), bf16),
        pltpu.VMEM((d, s), f32),
        pltpu.VMEM((d, _VR * len(_VSTEPS), _LANES), f32),
    ]
    hbm = pl.BlockSpec(memory_space=pl.ANY)
    out = pl.pallas_call(
        functools.partial(_kernel, n_heads=h),
        in_specs=[pl.BlockSpec(memory_space=pltpu.VMEM), hbm, hbm, hbm],
        out_specs=hbm,
        out_shape=jax.ShapeDtypeStruct((n, d, s), q.dtype),
        scratch_shapes=(
            slot + slot
            + [pltpu.VMEM((8, _LANES), i32), pltpu.VMEM((h, _LANES), f32)]
            + [pltpu.VMEM((n + _AHEAD * _G, d, s), q.dtype)] * 3
            + [pltpu.VMEM((n, d, s), q.dtype)]
            + [pltpu.SemaphoreType.DMA((_AHEAD + 1,))] * 3
            + [pltpu.SemaphoreType.DMA((1,))]
        ),
        compiler_params=pltpu.CompilerParams(vmem_limit_bytes=100 << 20),
    )(t.reshape(1, h), transposed(q), transposed(k), transposed(v))
    return jnp.transpose(out.reshape(b, h, d, s), (0, 1, 3, 2))
```

```python
import functools

import jax
import jax.numpy as jnp
from jax import lax
import jax.experimental.pallas as pl
import jax.experimental.pallas.tpu as pltpu

_LOG2E = 1.4426950408889634
_EPS = 1e-6
_T_SAFE = 8.0
_G = 2
_BQ = 512
_BK = 128
_LOOK = 2
_VR = 16
_VSTEPS = (5, 10, 15)
_KB_PARTS = 2
_DMA_STEP = 8
_AHEAD = 3
_LANES = 128

f32, bf16, i32 = jnp.float32, jnp.bfloat16, jnp.int32


def _inv_norm(x):
    return 1.0 / (jnp.sqrt(jnp.sum(x * x, axis=0, keepdims=True)) + _EPS)


def _tie(never, token, operand):
    bits = jnp.where(never, pltpu.bitcast(token, i32), pltpu.bitcast(operand, i32))
    return pltpu.bitcast(bits, bf16)


def _prologue_parts(q_src, k_src, scale, slot, *, seq, dim, with_vpu=True):
    q_s, k_s, qf_s, kb_s = slot
    n_chunks = _LANES // dim
    chunk = seq // n_chunks

    def q_part(lo):
        x = q_src[:, lo:lo + _LANES].astype(f32)
        y = x * (scale() * _inv_norm(x))
        q_s[lo // _LANES] = y.astype(bf16)
        if with_vpu:
            qf_s[:, lo:lo + _LANES] = y
        return y[dim - 8:, :]

    def k_norm(state, r0, c):
        x = k_src[:, c * chunk + r0: c * chunk + r0 + _LANES].astype(f32)
        state[c] = x * _inv_norm(x)
        return state[c][dim - 8:, :]

    def k_transpose(state, r0):
        kt = jnp.concatenate([state.pop(c) for c in range(n_chunks)], axis=0).T
        state["kt"] = kt
        k_s[r0:r0 + _LANES, :] = kt.astype(bf16)
        return kt[_LANES - 8:, :]

    def k_broadcast(state, c, m, d0, d1):
        for d in range(d0, d1):
            col = c * dim + d
            val = jnp.broadcast_to(state["kt"][_BK - _VR:_BK, col:col + 1], (_VR, _LANES))
            kb_s[d, m * _VR:(m + 1) * _VR, :] = val
        return val[_VR - 8:, :]

    parts = [functools.partial(q_part, lo) for lo in range(0, seq, _LANES)]
    for r0 in range(0, chunk, _LANES):
        state = {}
        parts += [functools.partial(k_norm, state, r0, c) for c in range(n_chunks)]
        parts.append(functools.partial(k_transpose, state, r0))
        for c in range(n_chunks):
            step = (c * chunk + r0) // _BK
            if with_vpu and step in _VSTEPS:
                n = dim // _KB_PARTS
                parts += [functools.partial(k_broadcast, state, c, _VSTEPS.index(step),
                                            a * n, (a + 1) * n) for a in range(_KB_PARTS)]
    return parts


def _chunk_weights(qw, c, n_chunks):
    d, n = qw.shape
    parts = []
    if c > 0:
        parts.append(jnp.zeros((d * c, n), bf16))
    parts.append(qw)
    if c < n_chunks - 1:
        parts.append(jnp.zeros((d * (n_chunks - 1 - c), n), bf16))
    return jnp.concatenate(parts, axis=0) if len(parts) > 1 else qw


class _VpuLogits:
    def __init__(self, slot, q0, m, dim):
        self.qf_s, self.kb_s = slot[2], slot[3]
        self.q0, self.m = q0, m
        self.tiles = _BQ // _LANES
        self.todo = [(d, j) for d in range(dim) for j in range(self.tiles)]
        self.acc = [None] * self.tiles
        self.n_tokens = 0

    def advance(self, count):
        for d, j in self.todo[:count]:
            c0 = self.q0 + j * _LANES
            prod = self.kb_s[d, self.m * _VR:(self.m + 1) * _VR, :] * jnp.broadcast_to(
                self.qf_s[d:d + 1, c0:c0 + _LANES], (_VR, _LANES))
            self.acc[j] = prod if self.acc[j] is None else self.acc[j] + prod
        del self.todo[:count]

    def token(self):
        self.n_tokens += 1
        live = [a for a in self.acc if a is not None]
        half = self.n_tokens % 2
        return live[(self.n_tokens // 2) % len(live)][half * 8:(half + 1) * 8, :]

    def result(self):
        self.advance(len(self.todo))
        return jnp.concatenate(self.acc, axis=1)


class _Pacer:
    def __init__(self, jobs, n_slots):
        self.jobs = list(jobs)
        self.slots = n_slots
        self.rest = sum(len(job.todo) for job in self.jobs)

    def tie(self, never, operand):
        if self.rest <= 0 or self.slots <= 0:
            return operand
        count = -(-self.rest // self.slots)
        self.slots -= 1
        while count > 0 and self.jobs:
            job = self.jobs[0]
            n = min(count, len(job.todo))
            job.advance(n)
            count -= n
            self.rest -= n
            token = job.token() if (count == 0 or not job.todo) else None
            if not job.todo:
                self.jobs.pop(0)
            if count == 0:
                operand = _tie(never, token, operand)
        return operand


def _kernel(t_hbm, q_hbm, k_hbm, v_hbm, o_hbm,
            q_a, k_a, qf_a, kb_a, q_b, k_b, qf_b, kb_b, zero_s, scale_s, t_v,
            q_v, k_v, v_v, o_v, sem_q, sem_k, sem_v, sem_o, sem_0, *, n_heads):
    n, dim, seq = o_v.shape
    n_groups = n // _G
    n_chunks = _LANES // dim
    chunk = seq // n_chunks
    nq, nk = seq // _BQ, seq // _BK
    slots = [(q_a, k_a, qf_a, kb_a), (q_b, k_b, qf_b, kb_b)]

    def in_copies(c):
        sem = c % (_AHEAD + 1)
        copies = [pltpu.make_async_copy(
            v_hbm.at[pl.ds(jnp.minimum(c, n_groups - 1) * _G, _G)],
            v_v.at[pl.ds(c * _G, _G)], sem_v.at[sem])]
        for g in range(1, _G + 1):
            row = c * _G + g
            for hbm, vmem, sems in ((q_hbm, q_v, sem_q), (k_hbm, k_v, sem_k)):
                copies.append(pltpu.make_async_copy(
                    hbm.at[pl.ds(jnp.minimum(row, n - 1), 1)], vmem.at[pl.ds(row, 1)],
                    sems.at[sem]))
        return copies

    def out_copy(h):
        return pltpu.make_async_copy(o_v.at[pl.ds(h, 1)], o_hbm.at[pl.ds(h, 1)], sem_o.at[0])

    def start(copies):
        for cp in copies:
            cp.start()

    def wait(copies):
        for cp in copies:
            cp.wait()

    head0 = [pltpu.make_async_copy(hbm.at[pl.ds(0, 1)], vmem.at[pl.ds(0, 1)], sem_0.at[m])
             for m, (hbm, vmem) in enumerate(((q_hbm, q_v), (k_hbm, k_v)))]
    t_copy = pltpu.make_async_copy(t_hbm, t_v, sem_0.at[2])
    start([t_copy] + head0)
    for c in range(_AHEAD - 1):
        start(in_copies(c))
    zero_s[...] = jnp.zeros(zero_s.shape, i32)
    t_copy.wait()

    t_row = t_v[...].astype(f32)
    safe = jnp.max(jnp.abs(t_row)) <= _T_SAFE
    t_pad = jnp.concatenate([t_row, jnp.zeros((1, _LANES - n_heads), f32)], axis=1)
    scale_s[...] = jnp.broadcast_to(t_pad * _LOG2E, (_LANES, _LANES)).T[:n_heads, :]

    def scale_of(head):
        return lambda: scale_s[pl.ds(head % n_heads, 1), :]

    wait(head0)

    def fast_group(i, carry):
        wait(in_copies(i))
        never = zero_s[...] != 0
        steps = [(g, j, kb) for g in range(_G) for j in range(nq) for kb in range(nk)]

        tied = {}
        for g in range(_G):
            head = i * _G + g + 1
            parts = _prologue_parts(q_v.at[head], k_v.at[head], scale_of(head),
                                    slots[(g + 1) % 2], seq=seq, dim=dim)
            lo, hi = 1, nq * nk - _LOOK - 2
            for m, part in enumerate(parts):
                tied.setdefault(g * nq * nk + lo + (m * (hi - lo)) // len(parts),
                                []).append(part)

        jobs, pacers = {}, {}
        n_regs = sum((_BK - (_VR if kb in _VSTEPS else 0)) // 16 for kb in range(nk))
        for g in range(_G):
            for j in range(nq):
                for m, kb in enumerate(_VSTEPS):
                    jobs[g, j, kb] = _VpuLogits(slots[g % 2], j * _BQ, m, dim)
                pacers[g, j] = _Pacer([jobs[g, j, kb] for kb in _VSTEPS], n_regs)

        def qk(n_step):
            g, j, kb = steps[n_step]
            q_s, k_s = slots[g % 2][:2]
            c, off = divmod(kb * _BK, chunk)
            tiles = _BQ // _LANES
            qw = jnp.concatenate([q_s[j * tiles + a] for a in range(tiles)], axis=1)
            w = _chunk_weights(qw, c, n_chunks)
            tokens = [part() for part in tied.get(n_step, [])]
            regs = []
            for r in range((_BK - (_VR if kb in _VSTEPS else 0)) // 16):
                reg = pacers[g, j].tie(never, k_s[off + r * 16: off + (r + 1) * 16, :])
                if r < len(tokens):
                    reg = _tie(never, tokens[r], reg)
                regs.append(reg)
            return jnp.dot(jnp.concatenate(regs, axis=0), w, preferred_element_type=f32)

        pending = [qk(m) for m in range(_LOOK)]
        acc = l_acc = None
        for n_step, (g, j, kb) in enumerate(steps):
            if n_step + _LOOK < len(steps):
                pending.append(qk(n_step + _LOOK))
            s = pending.pop(0)
            if (g, j, kb) in jobs:
                s = jnp.concatenate([s, jobs[g, j, kb].result()], axis=0)
            p = jnp.exp2(s)
            l_part = jnp.sum(p.reshape(_BK // 8, 8, _BQ), axis=0)
            l_acc = l_part if kb == 0 else l_acc + l_part
            head = i * _G + g
            pv = jnp.dot(v_v[head, :, kb * _BK:(kb + 1) * _BK], p.astype(bf16),
                         preferred_element_type=f32)
            acc = pv if kb == 0 else acc + pv
            if kb == nk - 1:
                l_sum = jnp.sum(l_acc, axis=0, keepdims=True)
                o_v[head, :, j * _BQ:(j + 1) * _BQ] = (acc * (1.0 / l_sum)).astype(o_v.dtype)
                if j == nq - 1:
                    out_copy(head).start()
            if n_step == _DMA_STEP:
                start(in_copies(i + _AHEAD - 1))
        return carry

    @pl.when(safe)
    def _():
        for part in _prologue_parts(q_v.at[0], k_v.at[0], scale_of(0), slots[0],
                                    seq=seq, dim=dim):
            part()
        lax.fori_loop(0, n_groups, fast_group, 0)

    def safe_group(i, carry):
        wait(in_copies(i))
        start(in_copies(i + _AHEAD - 1))
        q_s, k_s = slots[0][:2]

        def one_head(head, carry):
            for part in _prologue_parts(q_v.at[head], k_v.at[head], scale_of(head),
                                        slots[0], seq=seq, dim=dim, with_vpu=False):
                part()

            def q_tile(j, carry):
                qw = q_s[j]

                def logits(c):
                    return jnp.dot(k_s[...], _chunk_weights(qw, c, n_chunks),
                                   preferred_element_type=f32)

                m = None
                for c in range(n_chunks):
                    m_c = jnp.max(logits(c), axis=0, keepdims=True)
                    m = m_c if m is None else jnp.maximum(m, m_c)
                acc = l_sum = None
                for c in range(n_chunks):
                    p = jnp.exp2(logits(c) - m)
                    l_c = jnp.sum(p, axis=0, keepdims=True)
                    pv = jnp.dot(v_v[head, :, c * chunk:(c + 1) * chunk], p.astype(bf16),
                                 preferred_element_type=f32)
                    l_sum = l_c if l_sum is None else l_sum + l_c
                    acc = pv if acc is None else acc + pv
                q0 = pl.multiple_of(j * _LANES, _LANES)
                o_v[head, :, pl.ds(q0, _LANES)] = (acc * (1.0 / l_sum)).astype(o_v.dtype)
                return carry

            lax.fori_loop(0, seq // _LANES, q_tile, 0)
            out_copy(head).start()
            return carry

        return lax.fori_loop(i * _G, (i + 1) * _G, one_head, carry)

    @pl.when(jnp.logical_not(safe))
    def _():
        lax.fori_loop(0, n_groups, safe_group, 0)

    for c in range(n_groups, n_groups + _AHEAD - 1):
        wait(in_copies(c))
    pltpu.make_async_copy(o_v, o_hbm, sem_o.at[0]).wait()


@jax.jit
def pallas_standalone__qk_norm__prompt_kernel(
    q: jax.Array,
    k: jax.Array,
    v: jax.Array,
    t: jax.Array,
):
    b, h, s, d = q.shape
    n = b * h
    assert n % _G == 0 and s % _BQ == 0 and (s * d // _LANES) % _LANES == 0 and h <= _LANES

    def transposed(x):
        return jnp.transpose(x, (0, 1, 3, 2)).reshape(n, d, s)

    slot = [
        pltpu.VMEM((s // _LANES, d, _LANES), bf16),
        pltpu.VMEM((s * d // _LANES, _LANES), bf16),
        pltpu.VMEM((d, s), f32),
        pltpu.VMEM((d, _VR * len(_VSTEPS), _LANES), f32),
    ]
    hbm = pl.BlockSpec(memory_space=pl.ANY)
    out = pl.pallas_call(
        functools.partial(_kernel, n_heads=h),
        in_specs=[hbm, hbm, hbm, hbm],
        out_specs=hbm,
        out_shape=jax.ShapeDtypeStruct((n, d, s), q.dtype),
        scratch_shapes=(
            slot + slot
            + [pltpu.VMEM((8, _LANES), i32), pltpu.VMEM((h, _LANES), f32),
               pltpu.VMEM((1, h), t.dtype)]
            + [pltpu.VMEM((n + _AHEAD * _G, d, s), q.dtype)] * 3
            + [pltpu.VMEM((n, d, s), q.dtype)]
            + [pltpu.SemaphoreType.DMA((_AHEAD + 1,))] * 3
            + [pltpu.SemaphoreType.DMA((1,)), pltpu.SemaphoreType.DMA((3,))]
        ),
        compiler_params=pltpu.CompilerParams(vmem_limit_bytes=100 << 20),
    )(t.reshape(1, h), transposed(q), transposed(k), transposed(v))
    return jnp.transpose(out.reshape(b, h, d, s), (0, 1, 3, 2))
```

```python
import functools

import jax
import jax.numpy as jnp
from jax import lax
import jax.experimental.pallas as pl
import jax.experimental.pallas.tpu as pltpu

_LOG2E = 1.4426950408889634
_EPS = 1e-6
_T_SAFE = 8.0
_V_EXP_CLAMP = 100
_G = 2
_BQ = 512
_BK = 128
_LOOK = 2
_VR = 16
_VSTEPS = (5, 10, 15)
_KB_PARTS = 2
_DMA_STEP = 8
_AHEAD = 3
_LANES = 128

f32, bf16, i32 = jnp.float32, jnp.bfloat16, jnp.int32


def _inv_norm(x):
    return 1.0 / (jnp.sqrt(jnp.sum(x * x, axis=0, keepdims=True)) + _EPS)


def _tie(never, token, operand):
    bits = jnp.where(never, pltpu.bitcast(token, i32), pltpu.bitcast(operand, i32))
    return pltpu.bitcast(bits, bf16)


def _prologue_parts(q_src, k_src, v_src, scale, slot, *, seq, dim, with_vpu=True):
    q_s, k_s, qf_s, kb_s, v_s, vs_s = slot
    n_chunks = _LANES // dim
    chunk = seq // n_chunks

    def q_part(lo):
        x = q_src[:, lo:lo + _LANES].astype(f32)
        y = x * (scale() * _inv_norm(x))
        q_s[lo // _LANES] = y.astype(bf16)
        if with_vpu:
            qf_s[:, lo:lo + _LANES] = y
        return y[dim - 8:, :]

    def v_max(state, lo, hi):
        for c0 in range(lo, hi, _LANES):
            x = jnp.abs(v_src[:, c0:c0 + _LANES].astype(f32))
            state["m"] = jnp.maximum(state["m"], x) if "m" in state else x
        return state["m"][dim - 8:, :]

    def v_exponent(state):
        m = jnp.broadcast_to(jnp.max(state.pop("m"), axis=1, keepdims=True), (dim, _LANES))
        e = jnp.clip((pltpu.bitcast(m, i32) >> 23) - 127, -_V_EXP_CLAMP, _V_EXP_CLAMP)
        down = pltpu.bitcast((127 - e) << 23, f32)
        vs_s[0] = down
        vs_s[1] = pltpu.bitcast((127 + e) << 23, f32)
        return down[dim - 8:, :]

    def v_part(lo):
        y = v_src[:, lo:lo + _LANES].astype(f32) * vs_s[0]
        v_s[lo // _LANES] = y.astype(bf16)
        return y[dim - 8:, :]

    def k_norm(state, r0, c):
        x = k_src[:, c * chunk + r0: c * chunk + r0 + _LANES].astype(f32)
        state[c] = x * _inv_norm(x)
        return state[c][dim - 8:, :]

    def k_transpose(state, r0):
        kt = jnp.concatenate([state.pop(c) for c in range(n_chunks)], axis=0).T
        state["kt"] = kt
        k_s[r0:r0 + _LANES, :] = kt.astype(bf16)
        return kt[_LANES - 8:, :]

    def k_broadcast(state, c, m, d0, d1):
        for d in range(d0, d1):
            col = c * dim + d
            val = jnp.broadcast_to(state["kt"][_BK - _VR:_BK, col:col + 1], (_VR, _LANES))
            kb_s[d, m * _VR:(m + 1) * _VR, :] = val
        return val[_VR - 8:, :]

    parts = [functools.partial(q_part, lo) for lo in range(0, seq, _LANES)]
    for r0 in range(0, chunk, _LANES):
        state = {}
        parts += [functools.partial(k_norm, state, r0, c) for c in range(n_chunks)]
        parts.append(functools.partial(k_transpose, state, r0))
        for c in range(n_chunks):
            step = (c * chunk + r0) // _BK
            if with_vpu and step in _VSTEPS:
                n = dim // _KB_PARTS
                parts += [functools.partial(k_broadcast, state, c, _VSTEPS.index(step),
                                            a * n, (a + 1) * n) for a in range(_KB_PARTS)]
    if v_src is not None:
        state = {}
        parts += [functools.partial(v_max, state, lo, lo + seq // 4)
                  for lo in range(0, seq, seq // 4)]
        parts.append(functools.partial(v_exponent, state))
        parts += [functools.partial(v_part, lo) for lo in range(0, seq, _LANES)]
    return parts


def _chunk_weights(qw, c, n_chunks):
    d, n = qw.shape
    parts = []
    if c > 0:
        parts.append(jnp.zeros((d * c, n), bf16))
    parts.append(qw)
    if c < n_chunks - 1:
        parts.append(jnp.zeros((d * (n_chunks - 1 - c), n), bf16))
    return jnp.concatenate(parts, axis=0) if len(parts) > 1 else qw


class _VpuLogits:
    def __init__(self, slot, q0, m, dim):
        self.qf_s, self.kb_s = slot[2], slot[3]
        self.q0, self.m = q0, m
        self.tiles = _BQ // _LANES
        self.todo = [(d, j) for d in range(dim) for j in range(self.tiles)]
        self.acc = [None] * self.tiles
        self.n_tokens = 0

    def advance(self, count):
        for d, j in self.todo[:count]:
            c0 = self.q0 + j * _LANES
            prod = self.kb_s[d, self.m * _VR:(self.m + 1) * _VR, :] * jnp.broadcast_to(
                self.qf_s[d:d + 1, c0:c0 + _LANES], (_VR, _LANES))
            self.acc[j] = prod if self.acc[j] is None else self.acc[j] + prod
        del self.todo[:count]

    def token(self):
        self.n_tokens += 1
        live = [a for a in self.acc if a is not None]
        half = self.n_tokens % 2
        return live[(self.n_tokens // 2) % len(live)][half * 8:(half + 1) * 8, :]

    def result(self):
        self.advance(len(self.todo))
        return jnp.concatenate(self.acc, axis=1)


class _Pacer:
    def __init__(self, jobs, n_slots):
        self.jobs = list(jobs)
        self.slots = n_slots
        self.rest = sum(len(job.todo) for job in self.jobs)

    def tie(self, never, operand):
        if self.rest <= 0 or self.slots <= 0:
            return operand
        count = -(-self.rest // self.slots)
        self.slots -= 1
        while count > 0 and self.jobs:
            job = self.jobs[0]
            n = min(count, len(job.todo))
            job.advance(n)
            count -= n
            self.rest -= n
            token = job.token() if (count == 0 or not job.todo) else None
            if not job.todo:
                self.jobs.pop(0)
            if count == 0:
                operand = _tie(never, token, operand)
        return operand


def _kernel(t_hbm, q_hbm, k_hbm, v_hbm, o_hbm,
            q_a, k_a, qf_a, kb_a, v_a, vs_a, q_b, k_b, qf_b, kb_b, v_b, vs_b,
            zero_s, scale_s, t_v,
            q_v, k_v, v_v, o_v, sem_q, sem_k, sem_v, sem_o, sem_0, *, n_heads):
    n, dim, seq = o_v.shape
    n_groups = n // _G
    n_chunks = _LANES // dim
    chunk = seq // n_chunks
    nq, nk = seq // _BQ, seq // _BK
    assert _BK == _LANES
    slots = [(q_a, k_a, qf_a, kb_a, v_a, vs_a), (q_b, k_b, qf_b, kb_b, v_b, vs_b)]

    arrays = ((q_hbm, q_v, sem_q), (k_hbm, k_v, sem_k), (v_hbm, v_v, sem_v))

    def in_copies(c):
        sem = c % (_AHEAD + 1)
        copies = []
        for g in range(1, _G + 1):
            row = c * _G + g
            for hbm, vmem, sems in arrays:
                copies.append(pltpu.make_async_copy(
                    hbm.at[pl.ds(jnp.minimum(row, n - 1), 1)], vmem.at[pl.ds(row, 1)],
                    sems.at[sem]))
        return copies

    def out_copy(h):
        return pltpu.make_async_copy(o_v.at[pl.ds(h, 1)], o_hbm.at[pl.ds(h, 1)], sem_o.at[0])

    def start(copies):
        for cp in copies:
            cp.start()

    def wait(copies):
        for cp in copies:
            cp.wait()

    head0 = [pltpu.make_async_copy(hbm.at[pl.ds(0, 1)], vmem.at[pl.ds(0, 1)], sem_0.at[m])
             for m, (hbm, vmem, _) in enumerate(arrays)]
    t_copy = pltpu.make_async_copy(t_hbm, t_v, sem_0.at[3])
    start([t_copy] + head0)
    for c in range(_AHEAD - 1):
        start(in_copies(c))
    zero_s[...] = jnp.zeros(zero_s.shape, i32)
    t_copy.wait()

    t_row = t_v[...].astype(f32)
    safe = jnp.max(jnp.abs(t_row)) <= _T_SAFE
    t_pad = jnp.concatenate([t_row, jnp.zeros((1, _LANES - n_heads), f32)], axis=1)
    scale_s[...] = jnp.broadcast_to(t_pad * _LOG2E, (_LANES, _LANES)).T[:n_heads, :]

    def scale_of(head):
        return lambda: scale_s[pl.ds(head % n_heads, 1), :]

    wait(head0)

    def fast_group(i, carry):
        wait(in_copies(i))
        never = zero_s[...] != 0
        steps = [(g, j, kb) for g in range(_G) for j in range(nq) for kb in range(nk)]

        tied = {}
        for g in range(_G):
            head = i * _G + g + 1
            parts = _prologue_parts(q_v.at[head], k_v.at[head], v_v.at[head],
                                    scale_of(head), slots[(g + 1) % 2], seq=seq, dim=dim)
            lo, hi = 1, nq * nk - _LOOK - 2
            for m, part in enumerate(parts):
                tied.setdefault(g * nq * nk + lo + (m * (hi - lo)) // len(parts),
                                []).append(part)

        jobs, pacers = {}, {}
        n_regs = sum((_BK - (_VR if kb in _VSTEPS else 0)) // 16 for kb in range(nk))
        for g in range(_G):
            for j in range(nq):
                for m, kb in enumerate(_VSTEPS):
                    jobs[g, j, kb] = _VpuLogits(slots[g % 2], j * _BQ, m, dim)
                pacers[g, j] = _Pacer([jobs[g, j, kb] for kb in _VSTEPS], n_regs)

        def qk(n_step):
            g, j, kb = steps[n_step]
            q_s, k_s = slots[g % 2][:2]
            c, off = divmod(kb * _BK, chunk)
            tiles = _BQ // _LANES
            qw = jnp.concatenate([q_s[j * tiles + a] for a in range(tiles)], axis=1)
            w = _chunk_weights(qw, c, n_chunks)
            tokens = [part() for part in tied.get(n_step, [])]
            regs = []
            for r in range((_BK - (_VR if kb in _VSTEPS else 0)) // 16):
                reg = pacers[g, j].tie(never, k_s[off + r * 16: off + (r + 1) * 16, :])
                if r < len(tokens):
                    reg = _tie(never, tokens[r], reg)
                regs.append(reg)
            return jnp.dot(jnp.concatenate(regs, axis=0), w, preferred_element_type=f32)

        pending = [qk(m) for m in range(_LOOK)]
        acc = l_acc = None
        for n_step, (g, j, kb) in enumerate(steps):
            if n_step + _LOOK < len(steps):
                pending.append(qk(n_step + _LOOK))
            s = pending.pop(0)
            if (g, j, kb) in jobs:
                s = jnp.concatenate([s, jobs[g, j, kb].result()], axis=0)
            p = jnp.exp2(s)
            l_part = jnp.sum(p.reshape(_BK // 8, 8, _BQ), axis=0)
            l_acc = l_part if kb == 0 else l_acc + l_part
            head = i * _G + g
            pv = jnp.dot(slots[g % 2][4][kb], p.astype(bf16),
                         preferred_element_type=f32)
            acc = pv if kb == 0 else acc + pv
            if kb == nk - 1:
                l_sum = jnp.sum(l_acc, axis=0, keepdims=True)
                up = jnp.tile(slots[g % 2][5][1], (1, _BQ // _LANES))
                o_v[head, :, j * _BQ:(j + 1) * _BQ] = (
                    (acc * (1.0 / l_sum)) * up).astype(o_v.dtype)
                if j == nq - 1:
                    out_copy(head).start()
            if n_step == _DMA_STEP:
                start(in_copies(i + _AHEAD - 1))
        return carry

    @pl.when(safe)
    def _():
        for part in _prologue_parts(q_v.at[0], k_v.at[0], v_v.at[0], scale_of(0), slots[0],
                                    seq=seq, dim=dim):
            part()
        lax.fori_loop(0, n_groups, fast_group, 0)

    def safe_group(i, carry):
        wait(in_copies(i))
        start(in_copies(i + _AHEAD - 1))
        q_s, k_s = slots[0][:2]

        def one_head(head, carry):
            for part in _prologue_parts(q_v.at[head], k_v.at[head], None, scale_of(head),
                                        slots[0], seq=seq, dim=dim, with_vpu=False):
                part()

            def q_tile(j, carry):
                qw = q_s[j]

                def logits(c):
                    return jnp.dot(k_s[...], _chunk_weights(qw, c, n_chunks),
                                   preferred_element_type=f32)

                m = None
                for c in range(n_chunks):
                    m_c = jnp.max(logits(c), axis=0, keepdims=True)
                    m = m_c if m is None else jnp.maximum(m, m_c)
                acc = l_sum = None
                for c in range(n_chunks):
                    p = jnp.exp2(logits(c) - m)
                    l_c = jnp.sum(p, axis=0, keepdims=True)
                    pv = jnp.dot(v_v[head, :, c * chunk:(c + 1) * chunk], p.astype(bf16),
                                 preferred_element_type=f32)
                    l_sum = l_c if l_sum is None else l_sum + l_c
                    acc = pv if acc is None else acc + pv
                q0 = pl.multiple_of(j * _LANES, _LANES)
                o_v[head, :, pl.ds(q0, _LANES)] = (acc * (1.0 / l_sum)).astype(o_v.dtype)
                return carry

            lax.fori_loop(0, seq // _LANES, q_tile, 0)
            out_copy(head).start()
            return carry

        return lax.fori_loop(i * _G, (i + 1) * _G, one_head, carry)

    @pl.when(jnp.logical_not(safe))
    def _():
        lax.fori_loop(0, n_groups, safe_group, 0)

    for c in range(n_groups, n_groups + _AHEAD - 1):
        wait(in_copies(c))
    pltpu.make_async_copy(o_v, o_hbm, sem_o.at[0]).wait()


@jax.jit
def pallas_standalone__qk_norm__prompt_kernel(
    q: jax.Array,
    k: jax.Array,
    v: jax.Array,
    t: jax.Array,
):
    b, h, s, d = q.shape
    n = b * h
    assert n % _G == 0 and s % _BQ == 0 and (s * d // _LANES) % _LANES == 0 and h <= _LANES

    def transposed(x):
        return jnp.transpose(x, (0, 1, 3, 2)).reshape(n, d, s)

    slot = [
        pltpu.VMEM((s // _LANES, d, _LANES), bf16),
        pltpu.VMEM((s * d // _LANES, _LANES), bf16),
        pltpu.VMEM((d, s), f32),
        pltpu.VMEM((d, _VR * len(_VSTEPS), _LANES), f32),
        pltpu.VMEM((s // _LANES, d, _LANES), bf16),
        pltpu.VMEM((2, d, _LANES), f32),
    ]
    hbm = pl.BlockSpec(memory_space=pl.ANY)
    out = pl.pallas_call(
        functools.partial(_kernel, n_heads=h),
        in_specs=[hbm, hbm, hbm, hbm],
        out_specs=hbm,
        out_shape=jax.ShapeDtypeStruct((n, d, s), q.dtype),
        scratch_shapes=(
            slot + slot
            + [pltpu.VMEM((8, _LANES), i32), pltpu.VMEM((h, _LANES), f32),
               pltpu.VMEM((1, h), t.dtype)]
            + [pltpu.VMEM((n + _AHEAD * _G, d, s), q.dtype)] * 3
            + [pltpu.VMEM((n, d, s), q.dtype)]
            + [pltpu.SemaphoreType.DMA((_AHEAD + 1,))] * 3
            + [pltpu.SemaphoreType.DMA((1,)), pltpu.SemaphoreType.DMA((4,))]
        ),
        compiler_params=pltpu.CompilerParams(vmem_limit_bytes=100 << 20),
    )(t.reshape(1, h), transposed(q), transposed(k), transposed(v))
    return jnp.transpose(out.reshape(b, h, d, s), (0, 1, 3, 2))
```

```python
import functools

import jax
import jax.numpy as jnp
from jax import lax
import jax.experimental.pallas as pl
import jax.experimental.pallas.tpu as pltpu

_LOG2E = 1.4426950408889634
_EPS = 1e-6
_T_SAFE = 8.0
_V_EXP_CLAMP = 100
_G = 2
_BQ = 512
_BK = 128
_LOOK = 2
_VR = 16
_VSTEPS = (5, 10, 15)
_KB_PARTS = 2
_DMA_STEP = 124
_AHEAD = 3
_LANES = 128

f32, bf16, i32 = jnp.float32, jnp.bfloat16, jnp.int32


def _inv_norm(x):
    return 1.0 / (jnp.sqrt(jnp.sum(x * x, axis=0, keepdims=True)) + _EPS)


def _tie(never, token, operand):
    bits = jnp.where(never, pltpu.bitcast(token, i32), pltpu.bitcast(operand, i32))
    return pltpu.bitcast(bits, bf16)


def _prologue_parts(q_src, k_src, v_src, scale, slot, *, seq, dim, with_vpu=True):
    q_s, k_s, qf_s, kb_s, v_s, vs_s = slot
    n_chunks = _LANES // dim
    chunk = seq // n_chunks

    def q_part(lo):
        x = q_src[:, lo:lo + _LANES].astype(f32)
        y = x * (scale() * _inv_norm(x))
        q_s[lo // _LANES] = y.astype(bf16)
        if with_vpu:
            qf_s[:, lo:lo + _LANES] = y
        return y[dim - 8:, :]

    def v_max(state, lo):
        x = jnp.abs(v_src[:, lo:lo + _LANES].astype(f32))
        state["m"] = jnp.maximum(state["m"], x) if "m" in state else x
        return state["m"][dim - 8:, :]

    def v_exponent(state):
        m = jnp.broadcast_to(jnp.max(state.pop("m"), axis=1, keepdims=True), (dim, _LANES))
        e = jnp.clip((pltpu.bitcast(m, i32) >> 23) - 127, -_V_EXP_CLAMP, _V_EXP_CLAMP)
        down = pltpu.bitcast((127 - e) << 23, f32)
        vs_s[0] = down
        vs_s[1] = pltpu.bitcast((127 + e) << 23, f32)
        return down[dim - 8:, :]

    def v_part(lo):
        y = v_src[:, lo:lo + _LANES].astype(f32) * vs_s[0]
        v_s[lo // _LANES] = y.astype(bf16)
        return y[dim - 8:, :]

    def k_norm(state, r0, c):
        x = k_src[:, c * chunk + r0: c * chunk + r0 + _LANES].astype(f32)
        state[c] = x * _inv_norm(x)
        return state[c][dim - 8:, :]

    def k_transpose(state, r0):
        kt = jnp.concatenate([state.pop(c) for c in range(n_chunks)], axis=0).T
        state["kt"] = kt
        k_s[r0:r0 + _LANES, :] = kt.astype(bf16)
        return kt[_LANES - 8:, :]

    def k_broadcast(state, c, m, d0, d1):
        for d in range(d0, d1):
            col = c * dim + d
            val = jnp.broadcast_to(state["kt"][_BK - _VR:_BK, col:col + 1], (_VR, _LANES))
            kb_s[d, m * _VR:(m + 1) * _VR, :] = val
        return val[_VR - 8:, :]

    q_parts = [functools.partial(q_part, lo) for lo in range(0, seq, _LANES)]
    parts = []
    for r0 in range(0, chunk, _LANES):
        state = {}
        parts += [functools.partial(k_norm, state, r0, c) for c in range(n_chunks)]
        parts.append(functools.partial(k_transpose, state, r0))
        for c in range(n_chunks):
            step = (c * chunk + r0) // _BK
            if with_vpu and step in _VSTEPS:
                n = dim // _KB_PARTS
                parts += [functools.partial(k_broadcast, state, c, _VSTEPS.index(step),
                                            a * n, (a + 1) * n) for a in range(_KB_PARTS)]
    if v_src is None:
        return q_parts + parts
    state = {}
    m_parts = [functools.partial(v_max, state, lo) for lo in range(0, seq, _LANES)]
    m_parts.append(functools.partial(v_exponent, state))
    v_parts = [functools.partial(v_part, lo) for lo in range(0, seq, _LANES)]
    return m_parts + q_parts + v_parts + parts


def _chunk_weights(qw, c, n_chunks):
    d, n = qw.shape
    parts = []
    if c > 0:
        parts.append(jnp.zeros((d * c, n), bf16))
    parts.append(qw)
    if c < n_chunks - 1:
        parts.append(jnp.zeros((d * (n_chunks - 1 - c), n), bf16))
    return jnp.concatenate(parts, axis=0) if len(parts) > 1 else qw


class _VpuLogits:
    def __init__(self, slot, q0, m, dim):
        self.qf_s, self.kb_s = slot[2], slot[3]
        self.q0, self.m = q0, m
        self.tiles = _BQ // _LANES
        self.todo = [(d, j) for d in range(dim) for j in range(self.tiles)]
        self.acc = [None] * self.tiles
        self.n_tokens = 3

    def advance(self, count):
        for d, j in self.todo[:count]:
            c0 = self.q0 + j * _LANES
            prod = self.kb_s[d, self.m * _VR:(self.m + 1) * _VR, :] * jnp.broadcast_to(
                self.qf_s[d:d + 1, c0:c0 + _LANES], (_VR, _LANES))
            self.acc[j] = prod if self.acc[j] is None else self.acc[j] + prod
        del self.todo[:count]

    def token(self):
        self.n_tokens += 1
        live = [a for a in self.acc if a is not None]
        half = self.n_tokens % 2
        return live[(self.n_tokens // 2) % len(live)][half * 8:(half + 1) * 8, :]

    def result(self):
        self.advance(len(self.todo))
        return jnp.concatenate(self.acc, axis=1)


class _Pacer:
    def __init__(self, jobs, n_slots):
        self.jobs = list(jobs)
        self.slots = n_slots
        self.rest = sum(len(job.todo) for job in self.jobs)

    def tie(self, never, operand):
        if self.rest <= 0 or self.slots <= 0:
            return operand
        count = -(-self.rest // self.slots)
        self.slots -= 1
        while count > 0 and self.jobs:
            job = self.jobs[0]
            n = min(count, len(job.todo))
            job.advance(n)
            count -= n
            self.rest -= n
            token = job.token() if (count == 0 or not job.todo) else None
            if not job.todo:
                self.jobs.pop(0)
            if count == 0:
                operand = _tie(never, token, operand)
        return operand


def _kernel(t_hbm, q_hbm, k_hbm, v_hbm, o_hbm,
            q_a, k_a, qf_a, kb_a, v_a, vs_a, q_b, k_b, qf_b, kb_b, v_b, vs_b,
            zero_s, scale_s, t_v,
            q_v, k_v, v_v, o_v, sem_q, sem_k, sem_v, sem_o, sem_0, *, n_heads):
    n, dim, seq = o_v.shape
    n_groups = n // _G
    n_chunks = _LANES // dim
    chunk = seq // n_chunks
    nq, nk = seq // _BQ, seq // _BK
    assert _BK == _LANES
    slots = [(q_a, k_a, qf_a, kb_a, v_a, vs_a), (q_b, k_b, qf_b, kb_b, v_b, vs_b)]

    arrays = ((q_hbm, q_v, sem_q), (k_hbm, k_v, sem_k), (v_hbm, v_v, sem_v))

    def in_copies(c):
        sem = c % (_AHEAD + 1)
        copies = []
        for g in range(1, _G + 1):
            row = c * _G + g
            for hbm, vmem, sems in arrays:
                copies.append(pltpu.make_async_copy(
                    hbm.at[pl.ds(jnp.minimum(row, n - 1), 1)], vmem.at[pl.ds(row, 1)],
                    sems.at[sem]))
        return copies

    def out_copy(h):
        return pltpu.make_async_copy(o_v.at[pl.ds(h, 1)], o_hbm.at[pl.ds(h, 1)], sem_o.at[0])

    def start(copies):
        for cp in copies:
            cp.start()

    def wait(copies):
        for cp in copies:
            cp.wait()

    head0 = [pltpu.make_async_copy(hbm.at[pl.ds(0, 1)], vmem.at[pl.ds(0, 1)], sem_0.at[m])
             for m, (hbm, vmem, _) in enumerate(arrays)]
    t_copy = pltpu.make_async_copy(t_hbm, t_v, sem_0.at[3])
    start([t_copy] + head0)
    for c in range(_AHEAD - 1):
        start(in_copies(c))
    zero_s[...] = jnp.zeros(zero_s.shape, i32)
    t_copy.wait()

    t_row = t_v[...].astype(f32)
    safe = jnp.max(jnp.abs(t_row)) <= _T_SAFE
    t_pad = jnp.concatenate([t_row, jnp.zeros((1, _LANES - n_heads), f32)], axis=1)
    scale_s[...] = jnp.broadcast_to(t_pad * _LOG2E, (_LANES, _LANES)).T[:n_heads, :]

    def scale_of(head):
        return lambda: scale_s[pl.ds(head % n_heads, 1), :]

    wait(head0)

    def fast_group(i, carry):
        wait(in_copies(i))
        never = zero_s[...] != 0
        steps = [(g, j, kb) for g in range(_G) for j in range(nq) for kb in range(nk)]

        tied = {}
        for g in range(_G):
            head = i * _G + g + 1
            parts = _prologue_parts(q_v.at[head], k_v.at[head], v_v.at[head],
                                    scale_of(head), slots[(g + 1) % 2], seq=seq, dim=dim)
            lo, hi = 1, nq * nk - _LOOK - 2
            for m, part in enumerate(parts):
                tied.setdefault(g * nq * nk + lo + (m * (hi - lo)) // len(parts),
                                []).append(part)

        jobs, pacers = {}, {}
        n_regs = sum((_BK - (_VR if kb in _VSTEPS else 0)) // 16 for kb in range(nk))
        for g in range(_G):
            for j in range(nq):
                for m, kb in enumerate(_VSTEPS):
                    jobs[g, j, kb] = _VpuLogits(slots[g % 2], j * _BQ, m, dim)
                pacers[g, j] = _Pacer([jobs[g, j, kb] for kb in _VSTEPS], n_regs)

        def qk(n_step):
            g, j, kb = steps[n_step]
            q_s, k_s = slots[g % 2][:2]
            c, off = divmod(kb * _BK, chunk)
            tiles = _BQ // _LANES
            qw = jnp.concatenate([q_s[j * tiles + a] for a in range(tiles)], axis=1)
            w = _chunk_weights(qw, c, n_chunks)
            tokens = [part() for part in tied.get(n_step, [])]
            regs = []
            for r in range((_BK - (_VR if kb in _VSTEPS else 0)) // 16):
                reg = pacers[g, j].tie(never, k_s[off + r * 16: off + (r + 1) * 16, :])
                if r < len(tokens):
                    reg = _tie(never, tokens[r], reg)
                regs.append(reg)
            return jnp.dot(jnp.concatenate(regs, axis=0), w, preferred_element_type=f32)

        pending = [qk(m) for m in range(_LOOK)]
        acc = l_acc = None
        for n_step, (g, j, kb) in enumerate(steps):
            if n_step + _LOOK < len(steps):
                pending.append(qk(n_step + _LOOK))
            s = pending.pop(0)
            if (g, j, kb) in jobs:
                s = jnp.concatenate([s, jobs[g, j, kb].result()], axis=0)
            p = jnp.exp2(s)
            l_part = jnp.sum(p.reshape(_BK // 8, 8, _BQ), axis=0)
            l_acc = l_part if kb == 0 else l_acc + l_part
            head = i * _G + g
            pv = jnp.dot(slots[g % 2][4][kb], p.astype(bf16),
                         preferred_element_type=f32)
            acc = pv if kb == 0 else acc + pv
            if kb == nk - 1:
                l_sum = jnp.sum(l_acc, axis=0, keepdims=True)
                up = jnp.tile(slots[g % 2][5][1], (1, _BQ // _LANES))
                o_v[head, :, j * _BQ:(j + 1) * _BQ] = (
                    acc * ((1.0 / l_sum) * up)).astype(o_v.dtype)
                if j == nq - 1:
                    out_copy(head).start()
            if n_step == _DMA_STEP:
                start(in_copies(i + _AHEAD - 1))
        return carry

    @pl.when(safe)
    def _():
        for part in _prologue_parts(q_v.at[0], k_v.at[0], v_v.at[0], scale_of(0), slots[0],
                                    seq=seq, dim=dim):
            part()
        lax.fori_loop(0, n_groups, fast_group, 0)

    def safe_group(i, carry):
        wait(in_copies(i))
        start(in_copies(i + _AHEAD - 1))
        q_s, k_s = slots[0][:2]

        def one_head(head, carry):
            for part in _prologue_parts(q_v.at[head], k_v.at[head], None, scale_of(head),
                                        slots[0], seq=seq, dim=dim, with_vpu=False):
                part()

            def q_tile(j, carry):
                qw = q_s[j]

                def logits(c):
                    return jnp.dot(k_s[...], _chunk_weights(qw, c, n_chunks),
                                   preferred_element_type=f32)

                m = None
                for c in range(n_chunks):
                    m_c = jnp.max(logits(c), axis=0, keepdims=True)
                    m = m_c if m is None else jnp.maximum(m, m_c)
                acc = l_sum = None
                for c in range(n_chunks):
                    p = jnp.exp2(logits(c) - m)
                    l_c = jnp.sum(p, axis=0, keepdims=True)
                    pv = jnp.dot(v_v[head, :, c * chunk:(c + 1) * chunk], p.astype(bf16),
                                 preferred_element_type=f32)
                    l_sum = l_c if l_sum is None else l_sum + l_c
                    acc = pv if acc is None else acc + pv
                q0 = pl.multiple_of(j * _LANES, _LANES)
                o_v[head, :, pl.ds(q0, _LANES)] = (acc * (1.0 / l_sum)).astype(o_v.dtype)
                return carry

            lax.fori_loop(0, seq // _LANES, q_tile, 0)
            out_copy(head).start()
            return carry

        return lax.fori_loop(i * _G, (i + 1) * _G, one_head, carry)

    @pl.when(jnp.logical_not(safe))
    def _():
        lax.fori_loop(0, n_groups, safe_group, 0)

    for c in range(n_groups, n_groups + _AHEAD - 1):
        wait(in_copies(c))
    pltpu.make_async_copy(o_v, o_hbm, sem_o.at[0]).wait()


@jax.jit
def pallas_standalone__qk_norm__prompt_kernel(
    q: jax.Array,
    k: jax.Array,
    v: jax.Array,
    t: jax.Array,
):
    b, h, s, d = q.shape
    n = b * h
    assert n % _G == 0 and s % _BQ == 0 and (s * d // _LANES) % _LANES == 0 and h <= _LANES

    def transposed(x):
        return jnp.transpose(x, (0, 1, 3, 2)).reshape(n, d, s)

    slot = [
        pltpu.VMEM((s // _LANES, d, _LANES), bf16),
        pltpu.VMEM((s * d // _LANES, _LANES), bf16),
        pltpu.VMEM((d, s), f32),
        pltpu.VMEM((d, _VR * len(_VSTEPS), _LANES), f32),
        pltpu.VMEM((s // _LANES, d, _LANES), bf16),
        pltpu.VMEM((2, d, _LANES), f32),
    ]
    hbm = pl.BlockSpec(memory_space=pl.ANY)
    out = pl.pallas_call(
        functools.partial(_kernel, n_heads=h),
        in_specs=[hbm, hbm, hbm, hbm],
        out_specs=hbm,
        out_shape=jax.ShapeDtypeStruct((n, d, s), q.dtype),
        scratch_shapes=(
            slot + slot
            + [pltpu.VMEM((8, _LANES), i32), pltpu.VMEM((h, _LANES), f32),
               pltpu.VMEM((1, h), t.dtype)]
            + [pltpu.VMEM((n + _AHEAD * _G, d, s), q.dtype)] * 3
            + [pltpu.VMEM((n, d, s), q.dtype)]
            + [pltpu.SemaphoreType.DMA((_AHEAD + 1,))] * 3
            + [pltpu.SemaphoreType.DMA((1,)), pltpu.SemaphoreType.DMA((4,))]
        ),
        compiler_params=pltpu.CompilerParams(vmem_limit_bytes=100 << 20),
    )(t.reshape(1, h), transposed(q), transposed(k), transposed(v))
    return jnp.transpose(out.reshape(b, h, d, s), (0, 1, 3, 2))
```
